```python
import os as _os
_os.environ.setdefault("JAX_PLATFORMS", "cpu")
import jax
import jax.numpy as jnp

def _softmax(x, axis=-1):
    return jax.nn.softmax(x, axis=axis)
def _gelu(x):
    return jax.nn.gelu(x, approximate=True)
def _silu(x):
    return jax.nn.silu(x)
def _sigmoid(x):
    return jax.nn.sigmoid(x)
def _layernorm(x, axis=-1, eps=1e-5):
    m = jnp.mean(x, axis=axis, keepdims=True)
    v = jnp.var(x, axis=axis, keepdims=True)
    return (x - m) / jnp.sqrt(v + eps)
def _scatter_add(tgt, idx, src, axis=0):
    return tgt.at[idx].add(src)
def _segment_sum(src, seg, n):
    return jax.ops.segment_sum(src, seg, n)
class _Rng:
    def __init__(self, key):
        self._k = key
    def _next(self):
        self._k, sub = jax.random.split(self._k)
        return sub
    def normal(self, shape):
        return jax.random.normal(self._next(), shape, dtype=jnp.bfloat16)
    def randint(self, lo, hi, shape):
        return jax.random.randint(self._next(), shape, lo, hi, dtype=jnp.int32)
    def uniform(self, shape, lo=0.0, hi=1.0):
        return jax.random.uniform(self._next(), shape, jnp.bfloat16, lo, hi)
    def permutation(self, n):
        return jax.random.permutation(self._next(), n)


kernel_name = 'concat_heads__mha_block_cached__gqa_block_cached__decode'

def setup_inputs():
    _rng = _Rng(jax.random.key(int.from_bytes(__import__("os").urandom(4), "little")))
    _w = (lambda a: (lambda t: t.astype(jnp.bfloat16) if jnp.issubdtype(t.dtype, jnp.floating) else t)(jnp.asarray(a)))
    def _A_setup():
        B, Sq, D = 1, 1, 512
        H, Sk, Dh = 32, 4096, 128
        return {
            "x": _w((lambda *s: _rng.normal(s) * 0.8)(B, Sq, D)),
            "k_cache": _w((lambda *s: _rng.normal(s) * 0.8)(B, H, Sk, Dh)),
            "v_cache": _w((lambda *s: _rng.normal(s) * 0.05)(B, H, Sk, Dh)),
            "wq": _w((lambda *s: _rng.normal(s) * 0.8)(D, H * Dh) * (D ** -0.5)),
            "wo": _w((lambda *s: _rng.normal(s) * 0.05)(H * Dh, D) * ((H * Dh) ** -0.5)),
        }
    _A_in = _A_setup()

    def _B_setup():
        B, Sq, D = 1, 1, 512
        Hq, Hkv, Sk, Dh = 32, 32, 4096, 128
        assert Hq % Hkv == 0, (Hq, Hkv)
        return {
            "x": _w((lambda *s: _rng.normal(s) * 0.8)(B, Sq, D)),
            "k_cache": _w((lambda *s: _rng.normal(s) * 0.8)(B, Hkv, Sk, Dh)),
            "v_cache": _w((lambda *s: _rng.normal(s) * 0.05)(B, Hkv, Sk, Dh)),
            "wq": _w((lambda *s: _rng.normal(s) * 0.8)(D, Hq * Dh) * (D ** -0.5)),
            "wo": _w((lambda *s: _rng.normal(s) * 0.05)(Hq * Dh, D) * ((Hq * Dh) ** -0.5)),
        }
    _B_in = _B_setup()

    return {
        "A_x": _A_in["x"],
        "A_k_cache": _A_in["k_cache"],
        "A_v_cache": _A_in["v_cache"],
        "A_wq": _A_in["wq"],
        "A_wo": _A_in["wo"],
        "B_x": _B_in["x"],
        "B_k_cache": _B_in["k_cache"],
        "B_v_cache": _B_in["v_cache"],
        "B_wq": _B_in["wq"],
        "B_wo": _B_in["wo"],
    }

def reference(A_x, A_k_cache, A_v_cache, A_wq, A_wo, B_x, B_k_cache, B_v_cache, B_wq, B_wo):
    def _A_ref(x, k_cache, v_cache, wq, wo):
        B, Sq, D = x.shape
        H, Dh = 32, 128
        q = (lambda x, *d: x.transpose(*d))((x @ wq).reshape(B, Sq, H, Dh), 0, 2, 1, 3)
        scores = jnp.einsum("bhqd,bhkd->bhqk", q, k_cache) * (Dh ** -0.5)
        p = _softmax(scores, axis=-1)
        o = jnp.einsum("bhqk,bhkd->bhqd", p, v_cache)
        return (lambda x, *d: x.transpose(*d))(o, 0, 2, 1, 3).reshape(B, Sq, H * Dh) @ wo

    def _B_ref(x, k_cache, v_cache, wq, wo):
        B, Sq, D = x.shape
        Hq, Dh = 32, 128
        Hkv = k_cache.shape[1]
        rep = Hq // Hkv
        q = (lambda x, *d: x.transpose(*d))((x @ wq).reshape(B, Sq, Hq, Dh), 0, 2, 1, 3)
        k = jnp.repeat(k_cache, rep, axis=1)
        v = jnp.repeat(v_cache, rep, axis=1)
        scores = jnp.einsum("bhqd,bhkd->bhqk", q, k) * (Dh ** -0.5)
        p = _softmax(scores, axis=-1)
        o = jnp.einsum("bhqk,bhkd->bhqd", p, v)
        return (lambda x, *d: x.transpose(*d))(o, 0, 2, 1, 3).reshape(B, Sq, Hq * Dh) @ wo

    a = _A_ref(A_x, A_k_cache, A_v_cache, A_wq, A_wo)
    b = _B_ref(B_x, B_k_cache, B_v_cache, B_wq, B_wo)
    return jnp.concatenate([a, b], axis=-1)
```

```python
import jax
import jax.numpy as jnp
from jax import lax
import jax.experimental.pallas as pl
import jax.experimental.pallas.tpu as pltpu

H, SK, DH, D = 32, 4096, 128, 512
SCALE = DH ** -0.5
DEPTH = 3
KV_SIZES = [208] * 16 + [192] * 4
WO_GROUPS = (2048, 1024, 512, 256, 128, 128)


def _split(total, c):
    out = [c] * (total // c)
    if total % c:
        out.append(total % c)
    return out


def _offs(sizes):
    o = 0
    for s in sizes:
        yield o, s
        o += s


def _kernel(ax, ak, av, awq, awo, bx, bk, bv, bwq, bwo, out_ref,
            kvbuf, wq_buf, wo_buf, x_buf, q_scr, o_scr, kv_sems, w_sems):
    def start_kv(k, v, h, slot):
        for o, r in _offs(KV_SIZES):
            pltpu.make_async_copy(k.at[0, h, pl.ds(o, r)], kvbuf.at[slot, 0, pl.ds(o, r)],
                                  kv_sems.at[slot]).start(priority=0)
            pltpu.make_async_copy(v.at[0, h, pl.ds(o, r)], kvbuf.at[slot, 1, pl.ds(o, r)],
                                  kv_sems.at[slot]).start(priority=1)

    def wait_kv(slot):
        pltpu.make_async_copy(kvbuf.at[slot], kvbuf.at[slot], kv_sems.at[slot]).wait()

    def start_wq(w, b):
        def body(i, _):
            for o, c in _offs((1408, 1408, 1280)):
                for p in (0, 1):
                    r = pl.multiple_of(i * 16 + p * (D // 2), 16)
                    pltpu.make_async_copy(w.at[pl.ds(r, 16), pl.ds(o, c)],
                                          wq_buf.at[b, pl.ds(r, 16), pl.ds(o, c)],
                                          w_sems.at[b]).start(priority=p)
        lax.fori_loop(0, D // 32, body, None)

    def wait_wq(b):
        pltpu.make_async_copy(wq_buf.at[b], wq_buf.at[b], w_sems.at[b]).wait()

    def start_wo(w, b, r0, rows, sem):
        half = rows // 2
        for o, r in _offs(_split(half, 48)):
            for p in (0, 1):
                s = r0 + p * half + o
                pltpu.make_async_copy(w.at[pl.ds(s, r)], wo_buf.at[b, pl.ds(s, r)], sem).start(priority=p)

    def wait_wo(b, r0, rows, sem):
        d = wo_buf.at[b, pl.ds(r0, rows)]
        pltpu.make_async_copy(d, d, sem).wait()

    def proj_q(b):
        x = jnp.broadcast_to(x_buf[b], (8, D))
        q = jnp.dot(x, wq_buf[b], preferred_element_type=jnp.float32)
        for h in range(H):
            q_scr[b, h] = q[:, h * DH:(h + 1) * DH]

    def head(b, h, slot):
        q = q_scr[b, h].astype(jnp.bfloat16)
        s = lax.dot_general(q, kvbuf[slot, 0], (((1,), (1,)), ((), ())),
                            preferred_element_type=jnp.float32) * SCALE
        m = jnp.max(s, axis=-1, keepdims=True)
        e = jnp.exp(s - m)
        l = jnp.sum(e, axis=-1, keepdims=True)
        o = jnp.dot(e.astype(jnp.bfloat16), kvbuf[slot, 1], preferred_element_type=jnp.float32)
        o_scr[b, h] = o / l

    def proj_o(b, r0, rows):
        o = jnp.concatenate([o_scr[b, h] for h in range(r0 // DH, (r0 + rows) // DH)], axis=-1)
        return jnp.dot(o.astype(jnp.bfloat16), wo_buf[b, pl.ds(r0, rows)],
                       preferred_element_type=jnp.float32)

    def nxt(slot):
        return jnp.where(slot == DEPTH - 1, 0, slot + 1)

    xc = [pltpu.make_async_copy(ax.at[0], x_buf.at[0], w_sems.at[2]),
          pltpu.make_async_copy(bx.at[0], x_buf.at[1], w_sems.at[2])]
    for c in xc:
        c.start()
    start_wq(awq, 0)
    lax.fori_loop(0, DEPTH, lambda i, _: start_kv(ak, av, i, i), None)
    for c in xc:
        c.wait()
    wait_wq(0)
    proj_q(0)
    start_wq(bwq, 1)

    def body_a(h, slot):
        wait_kv(slot)
        head(0, h, slot)
        start_kv(ak, av, h + DEPTH, slot)
        return nxt(slot)
    slot = lax.fori_loop(0, H - DEPTH, body_a, jnp.int32(0))

    def body_ab(i, slot):
        wait_kv(slot)
        head(0, H - DEPTH + i, slot)
        start_kv(bk, bv, i, slot)
        return nxt(slot)
    slot = lax.fori_loop(0, DEPTH, body_ab, slot)

    start_wo(awo, 0, 0, H * DH, w_sems.at[2])
    wait_wq(1)
    proj_q(1)

    def body_b(h, slot):
        wait_kv(slot)
        head(1, h, slot)
        start_kv(bk, bv, h + DEPTH, slot)
        return nxt(slot)
    slot = lax.fori_loop(0, H - DEPTH, body_b, slot)

    wait_wo(0, 0, H * DH, w_sems.at[2])
    out_ref[0, :, pl.ds(0, D)] = proj_o(0, 0, H * DH)[0:1].astype(out_ref.dtype)
    for g, (r0, rows) in enumerate(_offs(WO_GROUPS)):
        start_wo(bwo, 1, r0, rows, w_sems.at[3 + g])

    def body_t(i, slot):
        wait_kv(slot)
        head(1, H - DEPTH + i, slot)
        return nxt(slot)
    lax.fori_loop(0, DEPTH, body_t, slot)

    acc = None
    for g, (r0, rows) in enumerate(_offs(WO_GROUPS)):
        wait_wo(1, r0, rows, w_sems.at[3 + g])
        t = proj_o(1, r0, rows)
        acc = t if acc is None else acc + t
    out_ref[0, :, pl.ds(D, D)] = acc[0:1].astype(out_ref.dtype)


@jax.jit
def pallas_concat_heads__mha_block_cached__gqa_block_cached__decode_kernel(
    A_x: jax.Array,
    A_k_cache: jax.Array,
    A_v_cache: jax.Array,
    A_wq: jax.Array,
    A_wo: jax.Array,
    B_x: jax.Array,
    B_k_cache: jax.Array,
    B_v_cache: jax.Array,
    B_wq: jax.Array,
    B_wo: jax.Array,
):
    return pl.pallas_call(
        _kernel,
        out_shape=jax.ShapeDtypeStruct((1, 1, 2 * D), A_x.dtype),
        in_specs=[pl.BlockSpec(memory_space=pltpu.HBM)] * 10,
        out_specs=pl.BlockSpec(memory_space=pltpu.VMEM),
        scratch_shapes=[
            pltpu.VMEM((DEPTH, 2, SK, DH), jnp.bfloat16),
            pltpu.VMEM((2, D, H * DH), jnp.bfloat16),
            pltpu.VMEM((2, H * DH, D), jnp.bfloat16),
            pltpu.VMEM((2, 1, D), jnp.bfloat16),
            pltpu.VMEM((2, H, 8, DH), jnp.float32),
            pltpu.VMEM((2, H, 8, DH), jnp.float32),
            pltpu.SemaphoreType.DMA((DEPTH,)),
            pltpu.SemaphoreType.DMA((3 + len(WO_GROUPS),)),
        ],
        compiler_params=pltpu.CompilerParams(
            vmem_limit_bytes=100 * 1024 * 1024,
            disable_bounds_checks=True,
            disable_semaphore_checks=True,
        ),
    )(A_x, A_k_cache, A_v_cache, A_wq, A_wo, B_x, B_k_cache, B_v_cache, B_wq, B_wo)
```

```python
import jax
import jax.numpy as jnp
from jax import lax
import jax.experimental.pallas as pl
import jax.experimental.pallas.tpu as pltpu

H, SK, DH, D = 32, 4096, 128, 512
SCALE = DH ** -0.5

G = 8
NG = H // G
T = 128
NT = SK // T
NU = NG * NT
LOOKAHEAD = 16
RING = 32
WS = 4
HS = H // WS
TAIL = 2

KV_COPIES = [(h, n, k + dk, 32)
             for k in (0, 64)
             for h, n in ((0, 3), (3, 2), (5, 1), (6, 2))
             for dk in (0, 32)]
W_RANGES = ((0, 2), (2, 2))


def _div(a, b):
    return lax.shift_right_logical(a, b.bit_length() - 1)


def _mod(a, b):
    return lax.bitwise_and(a, b - 1)


def _loop(lo, hi, body):
    lax.fori_loop(lo, hi, lambda i, _: body(i), None)


def _start(copies):
    for copy, priority in copies:
        copy.start(priority=priority)


def _wait_filled(ref, sem):
    pltpu.make_async_copy(ref, ref, sem).wait()


def _load_and_start(loads, copies):
    values, done = [], 0
    for i, load in enumerate(loads):
        values.append(load())
        upto = (i + 1) * len(copies) // len(loads) // 2 * 2
        _start(copies[done:upto])
        done = upto
    return values


def _own_rows(r):
    row = lax.broadcasted_iota(jnp.int32, (G, 128), 0)
    out = r[:, :128]
    for j in range(1, G):
        out = jnp.where(row == j, r[:, j * 128:(j + 1) * 128], out)
    return out


def _kernel(ax, ak, av, awq, awo, bx, bk, bv, bwq, bwo, out_ref,
            ring, wq_buf, wo_buf, x_buf, q_scr, s_scr, m_scr, l_scr, o_scr, y_scr,
            kv_sems, wq_sem, wo_sems):
    f32, bf16 = jnp.float32, jnp.bfloat16
    keys, values, wq, wo = (ak, bk), (av, bv), (awq, bwq), (awo, bwo)
    tail_rows = DH // TAIL

    def kv_copies(src, u):
        h0, k0, slot = _div(u, NT) * G, _mod(u, NT) * T, _mod(u, RING)
        return [(pltpu.make_async_copy(
                    src[b].at[0, pl.ds(h0 + h, n), pl.ds(pl.multiple_of(k0 + k, 32), c)],
                    ring.at[slot, b, pl.ds(h, n), pl.ds(k, c)],
                    kv_sems.at[_mod(u, LOOKAHEAD)]), b)
                for h, n, k, c in KV_COPIES for b in (0, 1)]

    def wq_copies(i, priorities=(0, 1)):
        rows = pl.ds(pl.multiple_of(i * 8, 8), 8)
        return [(pltpu.make_async_copy(
                    wq[b].at[pl.ds(s, n), rows, pl.ds(c, 1024)],
                    wq_buf.at[b, pl.ds(s, n), rows, pl.ds(c, 1024)],
                    wq_sem), priorities[b])
                for c in range(0, H * DH, 1024) for s, n in W_RANGES for b in (0, 1)]

    def wo_copies(i):
        step = HS * DH // LOOKAHEAD
        copies = []
        for dr in range(0, step, 16):
            r = pl.multiple_of(i * step + dr, 16)
            piece = 2 * _div(r, DH)
            last = 2 * HS - 1 + _div(r, tail_rows) - (HS - 1) * TAIL
            sem = (piece, jnp.where(r >= (HS - 1) * DH, last, piece + 1))
            copies += [(pltpu.make_async_copy(
                           wo[b].at[pl.ds(s, n), pl.ds(r, 16)],
                           wo_buf.at[b, pl.ds(s, n), pl.ds(r, 16)],
                           wo_sems.at[sem[b]]), b)
                       for s, n in W_RANGES for b in (0, 1)]
        return copies

    def unit_tiles(u, copies):
        slot = _mod(u, RING)
        tiles = _load_and_start(
            [lambda b=b, j=j: ring[slot, b, j] for b in (0, 1) for j in range(G)], copies)
        return tiles[:G], tiles[G:]

    def q_step(i, copies):
        b, g = _div(i, NG), _mod(i, NG)

        def head_columns(j):
            cols = pl.ds(pl.multiple_of((g * G + j) * DH, DH), DH)
            return wq_buf[b, :, :, cols].reshape(D, DH)

        w = _load_and_start([lambda j=j: head_columns(j) for j in range(G)], copies)
        x = jnp.broadcast_to(x_buf[b], (G, D))
        q_scr[b, g] = _own_rows(jnp.dot(x, jnp.concatenate(w, axis=1), preferred_element_type=f32))
        m_scr[b, g] = jnp.full((G, T), -jnp.inf, f32)

    def k_step(u, copies):
        _wait_filled(ring.at[_mod(u, RING)], kv_sems.at[_mod(u, LOOKAHEAD)])
        g = _div(u, NT)
        for b, k in enumerate(unit_tiles(u, copies)):
            r = lax.dot_general(q_scr[b, g].astype(bf16), jnp.concatenate(k, axis=0),
                                (((1,), (1,)), ((), ())), preferred_element_type=f32)
            s = _own_rows(r) * SCALE
            s_scr[u, b] = s
            m_scr[b, g] = jnp.maximum(m_scr[b, g], s)

    def v_step(u, copies):
        _wait_filled(ring.at[_mod(u, RING)], kv_sems.at[_mod(u, LOOKAHEAD)])
        g = _div(u, NT)
        e = [jnp.exp(s_scr[u, b] - m_scr[b, g]) for b in (0, 1)]
        for b, v in enumerate(unit_tiles(u, copies)):
            r = jnp.dot(e[b].astype(bf16), jnp.concatenate(v, axis=1), preferred_element_type=f32)
            l_scr[b, g] += e[b]
            o_scr[b, pl.ds(pl.multiple_of(g * G, G), G)] += _own_rows(r)

    def o_heads(b, t):
        return [jnp.broadcast_to(o_scr[b, pl.ds(s * HS + t, 1)], (8, DH)) for s in range(WS)]

    def o_step(i):
        t, b = _div(i, 2), _mod(i, 2)
        rows = pl.ds(pl.multiple_of(t * DH, DH), DH)
        _wait_filled(wo_buf.at[b, :, rows], wo_sems.at[i])
        o = jnp.concatenate(o_heads(b, t), axis=1).astype(bf16)
        y_scr[b] += jnp.dot(o, wo_buf[b, :, rows].reshape(WS * DH, D), preferred_element_type=f32)

    x_copies = [pltpu.make_async_copy(x.at[0], x_buf.at[b], wq_sem) for b, x in enumerate((ax, bx))]
    _loop(0, 2, lambda i: _start(wq_copies(i, priorities=(1, 1))))
    _loop(2, D // WS // 8, lambda i: _start(wq_copies(i)))
    for copy in x_copies:
        copy.start()
    early = LOOKAHEAD - 2 * NG
    _loop(0, early, lambda u: _start(kv_copies(keys, u)))
    for copy in x_copies:
        copy.wait()
    _wait_filled(wq_buf, wq_sem)
    _loop(0, 2 * NG, lambda i: q_step(i, kv_copies(keys, early + i)))

    _loop(0, NU - LOOKAHEAD, lambda u: k_step(u, kv_copies(keys, u + LOOKAHEAD)))
    _loop(NU - LOOKAHEAD, NU, lambda u: k_step(u, kv_copies(values, u + LOOKAHEAD - NU)))
    m_scr[...] = jnp.broadcast_to(jnp.max(m_scr[...], axis=-1, keepdims=True), m_scr.shape)
    l_scr[...] = jnp.zeros(l_scr.shape, f32)
    o_scr[...] = jnp.zeros(o_scr.shape, f32)

    _loop(0, NU - LOOKAHEAD, lambda u: v_step(u, kv_copies(values, u + LOOKAHEAD)))
    _loop(NU - LOOKAHEAD, NU, lambda u: v_step(u, wo_copies(u + LOOKAHEAD - NU)))
    o_scr[...] = o_scr[...] / jnp.sum(l_scr[...], axis=-1, keepdims=True).reshape(2, H, 1)

    y_scr[...] = jnp.zeros(y_scr.shape, f32)
    _loop(0, 2 * HS - 1, o_step)
    out_ref[0, :, :D] = y_scr[0, 0:1].astype(out_ref.dtype)
    y = y_scr[1]
    heads = o_heads(1, HS - 1)
    o = [jnp.concatenate([h[:, i * tail_rows:(i + 1) * tail_rows] for h in heads], axis=1).astype(bf16)
         for i in range(TAIL)]
    for i in range(TAIL):
        rows = pl.ds((HS - 1) * DH + i * tail_rows, tail_rows)
        _wait_filled(wo_buf.at[1, :, rows], wo_sems.at[2 * HS - 1 + i])
        y = y + jnp.dot(o[i], wo_buf[1, :, rows].reshape(WS * tail_rows, D),
                        preferred_element_type=f32)
    out_ref[0, :, D:] = y[0:1].astype(out_ref.dtype)


@jax.jit
def pallas_concat_heads__mha_block_cached__gqa_block_cached__decode_kernel(
    A_x: jax.Array,
    A_k_cache: jax.Array,
    A_v_cache: jax.Array,
    A_wq: jax.Array,
    A_wo: jax.Array,
    B_x: jax.Array,
    B_k_cache: jax.Array,
    B_v_cache: jax.Array,
    B_wq: jax.Array,
    B_wo: jax.Array,
):
    for cache in (A_k_cache, A_v_cache, B_k_cache, B_v_cache):
        assert cache.shape == (1, H, SK, DH), cache.shape
    f32, bf16 = jnp.float32, jnp.bfloat16
    wq_shape, wo_shape = (WS, D // WS, H * DH), (WS, HS * DH, D)
    return pl.pallas_call(
        _kernel,
        out_shape=jax.ShapeDtypeStruct((1, 1, 2 * D), A_x.dtype),
        in_specs=[pl.BlockSpec(memory_space=pltpu.HBM)] * 10,
        out_specs=pl.BlockSpec(memory_space=pltpu.VMEM),
        scratch_shapes=[
            pltpu.VMEM((RING, 2, G, T, DH), bf16),
            pltpu.VMEM((2, *wq_shape), bf16),
            pltpu.VMEM((2, *wo_shape), bf16),
            pltpu.VMEM((2, 1, D), bf16),
            pltpu.VMEM((2, NG, G, DH), f32),
            pltpu.VMEM((NU, 2, G, T), f32),
            pltpu.VMEM((2, NG, G, T), f32),
            pltpu.VMEM((2, NG, G, T), f32),
            pltpu.VMEM((2, H, DH), f32),
            pltpu.VMEM((2, 8, D), f32),
            pltpu.SemaphoreType.DMA((LOOKAHEAD,)),
            pltpu.SemaphoreType.DMA(()),
            pltpu.SemaphoreType.DMA((2 * HS - 1 + TAIL,)),
        ],
        compiler_params=pltpu.CompilerParams(
            vmem_limit_bytes=64 * 1024 * 1024,
            disable_bounds_checks=True,
            disable_semaphore_checks=True,
        ),
    )(A_x, A_k_cache, A_v_cache, A_wq.reshape(wq_shape), A_wo.reshape(wo_shape),
      B_x, B_k_cache, B_v_cache, B_wq.reshape(wq_shape), B_wo.reshape(wo_shape))
```

```python
import jax
import jax.numpy as jnp
from jax import lax
import jax.experimental.pallas as pl
import jax.experimental.pallas.tpu as pltpu

H, SK, DH, D = 32, 4096, 128, 512
SCALE = DH ** -0.5

G = 8
FIRST = 3
NG = H // G
T = 128
NT = SK // T
NU = NG * NT
LOOKAHEAD = 16
RING = 32
WS = 4
HS = H // WS
TAIL = 4

KV_COPIES = [(h, n, k, 64) for k in (0, 64) for h, n in ((0, 3), (3, 2), (5, 3))]
W_RANGES = ((0, 2), (2, 2))


def _div(a, b):
    return lax.shift_right_logical(a, b.bit_length() - 1)


def _mod(a, b):
    return lax.bitwise_and(a, b - 1)


def _loop(lo, hi, body):
    lax.fori_loop(lo, hi, lambda i, _: body(i), None)


def _start(copies):
    for copy, priority in copies:
        copy.start(priority=priority)


def _wait_filled(ref, sem):
    pltpu.make_async_copy(ref, ref, sem).wait()


def _load_and_start(loads, copies):
    values, done = [], 0
    for i, load in enumerate(loads):
        values.append(load())
        upto = (i + 1) * len(copies) // len(loads) // 2 * 2
        _start(copies[done:upto])
        done = upto
    return values


def _own_rows(r):
    row = lax.broadcasted_iota(jnp.int32, (G, 128), 0)
    out = r[:, :128]
    for j in range(1, G):
        out = jnp.where(row == j, r[:, j * 128:(j + 1) * 128], out)
    return out


def _kernel(ax, ak, av, awq, awo, bx, bk, bv, bwq, bwo, out_ref,
            ring, wq_buf, wo_buf, x_buf, q_scr, s_scr, m_scr, l_scr, o_scr, y_scr, col_scr,
            kv_sems, wq_sem, wo_sems):
    f32, bf16 = jnp.float32, jnp.bfloat16
    keys, values, wq, wo = (ak, bk), (av, bv), (awq, bwq), (awo, bwo)
    tail_rows = DH // TAIL

    def kv_copies(src, u):
        h0, k0, slot = FIRST + _div(u, NT) * G, _mod(u, NT) * T, _mod(u, RING)
        return [(pltpu.make_async_copy(
                    src[b].at[0, pl.ds(_mod(h0 + h, H), n), pl.ds(pl.multiple_of(k0 + k, 64), c)],
                    ring.at[slot, b, pl.ds(h, n), pl.ds(k, c)],
                    kv_sems.at[_mod(u, LOOKAHEAD)]), b)
                for h, n, k, c in KV_COPIES for b in (0, 1)]

    def wq_copies(i, priorities=(0, 1)):
        rows = pl.ds(pl.multiple_of(i * 8, 8), 8)
        return [(pltpu.make_async_copy(
                    wq[b].at[pl.ds(s, n), rows, pl.ds(c, 1024)],
                    wq_buf.at[b, pl.ds(s, n), rows, pl.ds(c, 1024)],
                    wq_sem), priorities[b])
                for c in range(0, H * DH, 1024) for s, n in W_RANGES for b in (0, 1)]

    def wo_copies(i):
        step = HS * DH // LOOKAHEAD
        copies = []
        for dr in range(0, step, 16):
            r = pl.multiple_of(i * step + dr, 16)
            piece = 2 * _div(r, DH)
            last = 2 * HS - 1 + _div(r, tail_rows) - (HS - 1) * TAIL
            sem = (piece, jnp.where(r >= (HS - 1) * DH, last, piece + 1))
            copies += [(pltpu.make_async_copy(
                           wo[b].at[pl.ds(s, n), pl.ds(r, 16)],
                           wo_buf.at[b, pl.ds(s, n), pl.ds(r, 16)],
                           wo_sems.at[sem[b]]), b)
                       for s, n in W_RANGES for b in (0, 1)]
        return copies

    def unit_tiles(u, copies):
        slot = _mod(u, RING)
        tiles = _load_and_start(
            [lambda b=b, j=j: ring[slot, b, j] for b in (0, 1) for j in range(G)], copies)
        return tiles[:G], tiles[G:]

    def q_step(i, copies):
        b, g = _div(i, NG), _mod(i, NG)

        def head_columns(j):
            cols = pl.ds(pl.multiple_of(_mod(FIRST + g * G + j, H) * DH, DH), DH)
            return wq_buf[b, :, :, cols].reshape(D, DH)

        w = _load_and_start([lambda j=j: head_columns(j) for j in range(G)], copies)
        x = jnp.broadcast_to(x_buf[b], (G, D))
        q_scr[b, g] = _own_rows(jnp.dot(x, jnp.concatenate(w, axis=1), preferred_element_type=f32))
        m_scr[b, g] = jnp.full((G, T), -jnp.inf, f32)

    def k_step(u, copies):
        _wait_filled(ring.at[_mod(u, RING)], kv_sems.at[_mod(u, LOOKAHEAD)])
        g = _div(u, NT)
        for b, k in enumerate(unit_tiles(u, copies)):
            r = lax.dot_general(q_scr[b, g].astype(bf16), jnp.concatenate(k, axis=0),
                                (((1,), (1,)), ((), ())), preferred_element_type=f32)
            s = _own_rows(r) * SCALE
            s_scr[u, b] = s
            m_scr[b, g] = jnp.maximum(m_scr[b, g], s)

    def v_step(u, copies):
        _wait_filled(ring.at[_mod(u, RING)], kv_sems.at[_mod(u, LOOKAHEAD)])
        g = _div(u, NT)
        e = [jnp.exp(s_scr[u, b] - m_scr[b, g]) for b in (0, 1)]
        for b, v in enumerate(unit_tiles(u, copies)):
            r = jnp.dot(e[b].astype(bf16), jnp.concatenate(v, axis=1), preferred_element_type=f32)
            l_scr[b, g] += e[b]
            o_scr[b, pl.ds(pl.multiple_of(g * G, G), G)] += _own_rows(r)

    def o_heads(b, t):
        return [jnp.broadcast_to(o_scr[b, pl.ds((s * HS + t + H - FIRST) & (H - 1), 1)], (8, DH))
                for s in range(WS)]

    def o_step(i):
        t, b = _div(i, 2), _mod(i, 2)
        rows = pl.ds(pl.multiple_of(t * DH, DH), DH)
        _wait_filled(wo_buf.at[b, :, rows], wo_sems.at[i])
        o = jnp.concatenate(o_heads(b, t), axis=1).astype(bf16)
        y_scr[b] += jnp.dot(o, wo_buf[b, :, rows].reshape(WS * DH, D), preferred_element_type=f32)

    x_copies = [pltpu.make_async_copy(x.at[0], x_buf.at[b], wq_sem) for b, x in enumerate((ax, bx))]
    _loop(0, 2, lambda i: _start(wq_copies(i, priorities=(1, 1))))
    _loop(2, D // WS // 8, lambda i: _start(wq_copies(i)))
    for copy in x_copies:
        copy.start()
    early = LOOKAHEAD - 2 * NG
    _loop(0, early, lambda u: _start(kv_copies(keys, u)))
    for copy in x_copies:
        copy.wait()
    _wait_filled(wq_buf, wq_sem)
    _loop(0, 2 * NG, lambda i: q_step(i, kv_copies(keys, early + i)))

    _loop(0, NU - LOOKAHEAD, lambda u: k_step(u, kv_copies(keys, u + LOOKAHEAD)))
    _loop(NU - LOOKAHEAD, NU, lambda u: k_step(u, kv_copies(values, u + LOOKAHEAD - NU)))
    m_scr[...] = jnp.broadcast_to(jnp.max(m_scr[...], axis=-1, keepdims=True), m_scr.shape)
    l_scr[...] = jnp.zeros(l_scr.shape, f32)
    o_scr[...] = jnp.zeros(o_scr.shape, f32)

    _loop(0, NU - LOOKAHEAD, lambda u: v_step(u, kv_copies(values, u + LOOKAHEAD)))
    _loop(NU - LOOKAHEAD, NU, lambda u: v_step(u, wo_copies(u + LOOKAHEAD - NU)))
    o_scr[...] = o_scr[...] / jnp.sum(l_scr[...], axis=-1, keepdims=True).reshape(2, H, 1)

    for s, o in enumerate(o_heads(1, HS - 1)):
        col_scr[s] = jnp.broadcast_to(o[0:1].astype(bf16).astype(f32), (DH, DH)).T
    y_scr[...] = jnp.zeros(y_scr.shape, f32)
    _loop(0, 2 * HS - 1, o_step)
    out_ref[0, :, :D] = y_scr[0, 0:1].astype(out_ref.dtype)
    y = jnp.where(lax.broadcasted_iota(jnp.int32, (8, D), 0) == 0, y_scr[1], 0.0)
    for i in range(TAIL):
        rows = pl.ds((HS - 1) * DH + i * tail_rows, tail_rows)
        _wait_filled(wo_buf.at[1, :, rows], wo_sems.at[2 * HS - 1 + i])
        o = col_scr[:, pl.ds(i * tail_rows, tail_rows)]
        p = wo_buf[1, :, rows].astype(f32) * jnp.concatenate([o] * (D // DH), axis=-1)
        y = y + jnp.sum(p.reshape(WS * tail_rows // 8, 8, D), axis=0)
    out_ref[0, :, D:] = jnp.sum(y, axis=0, keepdims=True).astype(out_ref.dtype)


@jax.jit
def pallas_concat_heads__mha_block_cached__gqa_block_cached__decode_kernel(
    A_x: jax.Array,
    A_k_cache: jax.Array,
    A_v_cache: jax.Array,
    A_wq: jax.Array,
    A_wo: jax.Array,
    B_x: jax.Array,
    B_k_cache: jax.Array,
    B_v_cache: jax.Array,
    B_wq: jax.Array,
    B_wo: jax.Array,
):
    for cache in (A_k_cache, A_v_cache, B_k_cache, B_v_cache):
        assert cache.shape == (1, H, SK, DH), cache.shape
    f32, bf16 = jnp.float32, jnp.bfloat16
    wq_shape, wo_shape = (WS, D // WS, H * DH), (WS, HS * DH, D)
    return pl.pallas_call(
        _kernel,
        out_shape=jax.ShapeDtypeStruct((1, 1, 2 * D), A_x.dtype),
        in_specs=[pl.BlockSpec(memory_space=pltpu.HBM)] * 10,
        out_specs=pl.BlockSpec(memory_space=pltpu.VMEM),
        scratch_shapes=[
            pltpu.VMEM((RING, 2, G, T, DH), bf16),
            pltpu.VMEM((2, *wq_shape), bf16),
            pltpu.VMEM((2, *wo_shape), bf16),
            pltpu.VMEM((2, 1, D), bf16),
            pltpu.VMEM((2, NG, G, DH), f32),
            pltpu.VMEM((NU, 2, G, T), f32),
            pltpu.VMEM((2, NG, G, T), f32),
            pltpu.VMEM((2, NG, G, T), f32),
            pltpu.VMEM((2, H, DH), f32),
            pltpu.VMEM((2, 8, D), f32),
            pltpu.VMEM((WS, DH, DH), f32),
            pltpu.SemaphoreType.DMA((LOOKAHEAD,)),
            pltpu.SemaphoreType.DMA(()),
            pltpu.SemaphoreType.DMA((2 * HS - 1 + TAIL,)),
        ],
        compiler_params=pltpu.CompilerParams(
            vmem_limit_bytes=64 * 1024 * 1024,
            disable_bounds_checks=True,
            disable_semaphore_checks=True,
        ),
    )(A_x, A_k_cache, A_v_cache, A_wq.reshape(wq_shape), A_wo.reshape(wo_shape),
      B_x, B_k_cache, B_v_cache, B_wq.reshape(wq_shape), B_wo.reshape(wo_shape))
```

```python
import jax
import jax.numpy as jnp
from jax import lax
import jax.experimental.pallas as pl
import jax.experimental.pallas.tpu as pltpu

H, SK, DH, D = 32, 4096, 128, 512
SCALE = DH ** -0.5

G = 8
FIRST = 3
NG = H // G
T = 128
NT = SK // T
NU = NG * NT
LOOKAHEAD = 16
RING = 32
WS = 4
HS = H // WS
TAIL = 4

KV_COPIES = [(h, n, k, 64) for k in (0, 64) for h, n in ((0, 3), (3, 2), (5, 3))]
assert G - FIRST in [h for h, _, _, _ in KV_COPIES]
W_RANGES = ((0, 2), (2, 2))


def _div(a, b):
    return lax.shift_right_logical(a, b.bit_length() - 1)


def _mod(a, b):
    return lax.bitwise_and(a, b - 1)


def _loop(lo, hi, body):
    lax.fori_loop(lo, hi, lambda i, _: body(i), None)


def _start(copies):
    for copy, priority in copies:
        copy.start(priority=priority)


def _wait_filled(ref, sem):
    pltpu.make_async_copy(ref, ref, sem).wait()


def _load_and_start(loads, copies):
    values, done = [], 0
    for i, load in enumerate(loads):
        values.append(load())
        upto = (i + 1) * len(copies) // len(loads) // 2 * 2
        _start(copies[done:upto])
        done = upto
    return values


def _own_rows(r):
    row = lax.broadcasted_iota(jnp.int32, (G, 128), 0)
    out = r[:, :128]
    for j in range(1, G):
        out = jnp.where(row == j, r[:, j * 128:(j + 1) * 128], out)
    return out


def _kernel(ax, ak, av, awq, awo, bx, bk, bv, bwq, bwo, out_ref,
            ring, wq_buf, wo_buf, x_buf, q_scr, s_scr, m_scr, l_scr, o_scr, y_scr,
            col_scr, kv_sems, x_sem, wq_sem, wo_sems):
    f32, bf16 = jnp.float32, jnp.bfloat16
    keys, values, wq, wo = (ak, bk), (av, bv), (awq, bwq), (awo, bwo)
    tail_rows = DH // TAIL

    def kv_copies(src, u):
        h0, k0, slot = FIRST + _div(u, NT) * G, _mod(u, NT) * T, _mod(u, RING)
        return [(pltpu.make_async_copy(
                    src[b].at[0, pl.ds(_mod(h0 + h, H), n), pl.ds(pl.multiple_of(k0 + k, c), c)],
                    ring.at[slot, b, pl.ds(h, n), pl.ds(k, c)],
                    kv_sems.at[_mod(u, LOOKAHEAD)]), b)
                for h, n, k, c in KV_COPIES for b in (0, 1)]

    def wq_copies(i, priorities=(0, 1)):
        rows = pl.ds(pl.multiple_of(i * 8, 8), 8)
        return [(pltpu.make_async_copy(
                    wq[b].at[pl.ds(s, n), rows, pl.ds(c, 1024)],
                    wq_buf.at[b, pl.ds(s, n), rows, pl.ds(c, 1024)],
                    wq_sem), priorities[b])
                for c in range(0, H * DH, 1024) for s, n in W_RANGES for b in (0, 1)]

    def wo_copies(i):
        step = HS * DH // LOOKAHEAD
        copies = []
        for dr in range(0, step, 16):
            r = pl.multiple_of(i * step + dr, 16)
            piece = 2 * _div(r, DH)
            last = 2 * HS - 1 + _div(r, tail_rows) - (HS - 1) * TAIL
            sem = (piece, jnp.where(r >= (HS - 1) * DH, last, piece + 1))
            copies += [(pltpu.make_async_copy(
                           wo[b].at[pl.ds(s, n), pl.ds(r, 16)],
                           wo_buf.at[b, pl.ds(s, n), pl.ds(r, 16)],
                           wo_sems.at[sem[b]]), b)
                       for s, n in W_RANGES for b in (0, 1)]
        return copies

    def unit_tiles(u, copies):
        slot = _mod(u, RING)
        tiles = _load_and_start(
            [lambda b=b, j=j: ring[slot, b, j] for b in (0, 1) for j in range(G)], copies)
        return tiles[:G], tiles[G:]

    def q_step(i, copies):
        b, g = _div(i, NG), _mod(i, NG)

        def head_columns(j):
            cols = pl.ds(pl.multiple_of(_mod(FIRST + g * G + j, H) * DH, DH), DH)
            return wq_buf[b, :, :, cols].reshape(D, DH)

        w = _load_and_start([lambda j=j: head_columns(j) for j in range(G)], copies)
        x = jnp.broadcast_to(x_buf[b], (G, D))
        q_scr[b, g] = _own_rows(jnp.dot(x, jnp.concatenate(w, axis=1), preferred_element_type=f32))
        m_scr[b, g] = jnp.full((G, T), -jnp.inf, f32)

    def k_step(u, copies):
        _wait_filled(ring.at[_mod(u, RING)], kv_sems.at[_mod(u, LOOKAHEAD)])
        g = _div(u, NT)
        for b, k in enumerate(unit_tiles(u, copies)):
            r = lax.dot_general(q_scr[b, g].astype(bf16), jnp.concatenate(k, axis=0),
                                (((1,), (1,)), ((), ())), preferred_element_type=f32)
            s = _own_rows(r) * SCALE
            s_scr[u, b] = s
            m_scr[b, g] = jnp.maximum(m_scr[b, g], s)

    def v_step(u, copies):
        _wait_filled(ring.at[_mod(u, RING)], kv_sems.at[_mod(u, LOOKAHEAD)])
        g = _div(u, NT)
        e = [jnp.exp(s_scr[u, b] - m_scr[b, g]) for b in (0, 1)]
        for b, v in enumerate(unit_tiles(u, copies)):
            r = jnp.dot(e[b].astype(bf16), jnp.concatenate(v, axis=1), preferred_element_type=f32)
            l_scr[b, g] += e[b]
            o_scr[b, pl.ds(pl.multiple_of(g * G, G), G)] += _own_rows(r)

    def o_heads(b, t):
        return [jnp.broadcast_to(o_scr[b, pl.ds((s * HS + t + H - FIRST) & (H - 1), 1)], (8, DH))
                for s in range(WS)]

    def o_step(i):
        t, b = _div(i, 2), _mod(i, 2)
        rows = pl.ds(pl.multiple_of(t * DH, DH), DH)
        _wait_filled(wo_buf.at[b, :, rows], wo_sems.at[i])
        o = jnp.concatenate(o_heads(b, t), axis=1).astype(bf16)
        y_scr[b] += jnp.dot(o, wo_buf[b, :, rows].reshape(WS * DH, D), preferred_element_type=f32)

    x_copies = [pltpu.make_async_copy(x.at[0], x_buf.at[b], x_sem) for b, x in enumerate((ax, bx))]
    _loop(0, 2, lambda i: _start(wq_copies(i, priorities=(1, 1))))
    _loop(2, D // WS // 8, lambda i: _start(wq_copies(i)))
    for copy in x_copies:
        copy.start()
    early = LOOKAHEAD - 2 * NG
    _loop(0, early, lambda u: _start(kv_copies(keys, u)))
    for copy in x_copies:
        copy.wait()
    _wait_filled(wq_buf, wq_sem)
    _loop(0, 2 * NG, lambda i: q_step(i, kv_copies(keys, early + i)))

    _loop(0, NU - LOOKAHEAD, lambda u: k_step(u, kv_copies(keys, u + LOOKAHEAD)))
    _loop(NU - LOOKAHEAD, NU, lambda u: k_step(u, kv_copies(values, u + LOOKAHEAD - NU)))
    m_scr[...] = jnp.broadcast_to(jnp.max(m_scr[...], axis=-1, keepdims=True), m_scr.shape)
    l_scr[...] = jnp.zeros(l_scr.shape, f32)
    o_scr[...] = jnp.zeros(o_scr.shape, f32)

    _loop(0, NU - LOOKAHEAD, lambda u: v_step(u, kv_copies(values, u + LOOKAHEAD)))
    _loop(NU - LOOKAHEAD, NU, lambda u: v_step(u, wo_copies(u + LOOKAHEAD - NU)))
    o_scr[...] = o_scr[...] / jnp.sum(l_scr[...], axis=-1, keepdims=True).reshape(2, H, 1)

    for s, o in enumerate(o_heads(1, HS - 1)):
        col_scr[s] = jnp.broadcast_to(o[0:1].astype(bf16).astype(f32), (DH, DH)).T
    y_scr[...] = jnp.zeros(y_scr.shape, f32)
    _loop(0, 2 * HS - 1, o_step)
    out_ref[0, :, :D] = y_scr[0, 0:1].astype(out_ref.dtype)
    y = jnp.where(lax.broadcasted_iota(jnp.int32, (8, D), 0) == 0, y_scr[1], 0.0)
    for i in range(TAIL):
        rows = pl.ds((HS - 1) * DH + i * tail_rows, tail_rows)
        _wait_filled(wo_buf.at[1, :, rows], wo_sems.at[2 * HS - 1 + i])
        o = col_scr[:, pl.ds(i * tail_rows, tail_rows)]
        p = wo_buf[1, :, rows].astype(f32) * jnp.concatenate([o] * (D // DH), axis=-1)
        y = y + jnp.sum(p.reshape(WS * tail_rows // 8, 8, D), axis=0)
    out_ref[0, :, D:] = jnp.sum(y, axis=0, keepdims=True).astype(out_ref.dtype)


@jax.jit
def pallas_concat_heads__mha_block_cached__gqa_block_cached__decode_kernel(
    A_x: jax.Array,
    A_k_cache: jax.Array,
    A_v_cache: jax.Array,
    A_wq: jax.Array,
    A_wo: jax.Array,
    B_x: jax.Array,
    B_k_cache: jax.Array,
    B_v_cache: jax.Array,
    B_wq: jax.Array,
    B_wo: jax.Array,
):
    for cache in (A_k_cache, A_v_cache, B_k_cache, B_v_cache):
        assert cache.shape == (1, H, SK, DH), cache.shape
    f32, bf16 = jnp.float32, jnp.bfloat16
    wq_shape, wo_shape = (WS, D // WS, H * DH), (WS, HS * DH, D)
    return pl.pallas_call(
        _kernel,
        out_shape=jax.ShapeDtypeStruct((1, 1, 2 * D), A_x.dtype),
        in_specs=[pl.BlockSpec(memory_space=pltpu.HBM)] * 10,
        out_specs=pl.BlockSpec(memory_space=pltpu.VMEM),
        scratch_shapes=[
            pltpu.VMEM((RING, 2, G, T, DH), bf16),
            pltpu.VMEM((2, *wq_shape), bf16),
            pltpu.VMEM((2, *wo_shape), bf16),
            pltpu.VMEM((2, 1, D), bf16),
            pltpu.VMEM((2, NG, G, DH), f32),
            pltpu.VMEM((NU, 2, G, T), f32),
            pltpu.VMEM((2, NG, G, T), f32),
            pltpu.VMEM((2, NG, G, T), f32),
            pltpu.VMEM((2, H, DH), f32),
            pltpu.VMEM((2, 8, D), f32),
            pltpu.VMEM((WS, DH, DH), f32),
            pltpu.SemaphoreType.DMA((LOOKAHEAD,)),
            pltpu.SemaphoreType.DMA(()),
            pltpu.SemaphoreType.DMA(()),
            pltpu.SemaphoreType.DMA((2 * HS - 1 + TAIL,)),
        ],
        compiler_params=pltpu.CompilerParams(
            vmem_limit_bytes=64 * 1024 * 1024,
            disable_semaphore_checks=True,
        ),
    )(A_x, A_k_cache, A_v_cache, A_wq.reshape(wq_shape), A_wo.reshape(wo_shape),
      B_x, B_k_cache, B_v_cache, B_wq.reshape(wq_shape), B_wo.reshape(wo_shape))
```
